```python
import jax
import jax.numpy as jnp

def _softmax(x, axis=-1):
    return jax.nn.softmax(x, axis=axis)
def _gelu(x):
    return jax.nn.gelu(x, approximate=True)
def _silu(x):
    return jax.nn.silu(x)
def _sigmoid(x):
    return jax.nn.sigmoid(x)
def _layernorm(x, axis=-1, eps=1e-5):
    m = jnp.mean(x, axis=axis, keepdims=True)
    v = jnp.var(x, axis=axis, keepdims=True)
    return (x - m) / jnp.sqrt(v + eps)
def _scatter_add(tgt, idx, src, axis=0):
    return tgt.at[idx].add(src)
def _segment_sum(src, seg, n):
    return jax.ops.segment_sum(src, seg, n)
class _Rng:
    def __init__(self, key):
        self._k = key
    def _next(self):
        self._k, sub = jax.random.split(self._k)
        return sub
    def normal(self, shape):
        return jax.random.normal(self._next(), shape, dtype=jnp.bfloat16)
    def randint(self, lo, hi, shape):
        return jax.random.randint(self._next(), shape, lo, hi, dtype=jnp.int32)
    def uniform(self, shape, lo=0.0, hi=1.0):
        return jax.random.uniform(self._next(), shape, jnp.bfloat16, lo, hi)
    def permutation(self, n):
        return jax.random.permutation(self._next(), n)


kernel_name = 'sequential_preLN__sliding_block_cached__glu_gated_swiglu__decode'

def setup_inputs():
    _rng = _Rng(jax.random.key(int.from_bytes(__import__("os").urandom(4), "little")))
    _w = (lambda a: (lambda t: t.astype(jnp.bfloat16) if jnp.issubdtype(t.dtype, jnp.floating) else t)(jnp.asarray(a)))
    def _A_setup():
        B, Sq, D = 1, 1, 640
        Hq, Hkv, Sk, Dh = 32, 32, 32768, 192
        assert Hq % Hkv == 0, (Hq, Hkv)
        return {
            "x": _w((lambda *s: _rng.normal(s) * 0.05)(B, Sq, D)),
            "k_cache": _w((lambda *s: _rng.normal(s) * 0.05)(B, Hkv, Sk, Dh)),
            "v_cache": _w((lambda *s: _rng.normal(s) * 0.05)(B, Hkv, Sk, Dh)),
            "wq": _w((lambda *s: _rng.normal(s) * 0.05)(D, Hq * Dh) * (D ** -0.5)),
            "wo": _w((lambda *s: _rng.normal(s) * 0.05)(Hq * Dh, D) * ((Hq * Dh) ** -0.5)),
        }
    _A_in = _A_setup()

    def _B_setup():
        B, S, D, F = 1, 1, 640, 1536
        return {
            "x": _w((lambda *s: _rng.normal(s) * 0.05)(B, S, D)),
            "w1": _w((lambda *s: _rng.normal(s) * 0.05)(D, F) * (2.0 / D) ** 0.5),
            "w3": _w((lambda *s: _rng.normal(s) * 0.05)(D, F) * (2.0 / D) ** 0.5),
            "w2": _w((lambda *s: _rng.normal(s) * 0.05)(F, D) * (2.0 / F) ** 0.5),
        }
    _B_in = _B_setup()

    return {
        "A_x": _A_in["x"],
        "A_k_cache": _A_in["k_cache"],
        "A_v_cache": _A_in["v_cache"],
        "A_wq": _A_in["wq"],
        "A_wo": _A_in["wo"],
        "B_x": _B_in["x"],
        "B_w1": _B_in["w1"],
        "B_w3": _B_in["w3"],
        "B_w2": _B_in["w2"],
    }

def reference(A_x, A_k_cache, A_v_cache, A_wq, A_wo, B_x, B_w1, B_w3, B_w2):
    def _A_ref(x, k_cache, v_cache, wq, wo):
        B, Sq, D = x.shape
        Hq, Dh = 32, 192
        Hkv, Sk = k_cache.shape[1], k_cache.shape[2]
        W = min(4096, max(256, Sk // 4))
        rep = Hq // Hkv
        q = (lambda x, *d: x.transpose(*d))((x @ wq).reshape(B, Sq, Hq, Dh), 0, 2, 1, 3)
        k = jnp.repeat(k_cache[:, :, Sk - W:, :], rep, axis=1)
        v = jnp.repeat(v_cache[:, :, Sk - W:, :], rep, axis=1)
        scores = jnp.einsum("bhqd,bhkd->bhqk", q, k) * (Dh ** -0.5)
        p = _softmax(scores, axis=-1)
        o = jnp.einsum("bhqk,bhkd->bhqd", p, v)
        return (lambda x, *d: x.transpose(*d))(o, 0, 2, 1, 3).reshape(B, Sq, Hq * Dh) @ wo

    def _B_ref(x, w1, w3, w2):
        gate = jnp.einsum("bsd,df->bsf", x, w1)
        up = jnp.einsum("bsd,df->bsf", x, w3)
        h = _silu(gate) * up
        out = jnp.einsum("bsf,fd->bsd", h, w2)
        return out

    x = A_x
    h = x + _A_ref(_layernorm(x, axis=-1), A_k_cache, A_v_cache, A_wq, A_wo)
    h2 = h + _B_ref(_layernorm(h, axis=-1), B_w1, B_w3, B_w2)
    return h2
```

```python
import jax
import jax.numpy as jnp
import numpy as np
from jax import lax
import jax.experimental.pallas as pl
import jax.experimental.pallas.tpu as pltpu

H, DH, SK, D, F = 32, 192, 32768, 640, 1536
W = min(4096, max(256, SK // 4))
BF = jnp.bfloat16
F32 = jnp.float32


def _bf16_round(v):
    u = int(np.float32(v).view(np.uint32))
    u = (u + 0x7FFF + ((u >> 16) & 1)) & 0xFFFF0000
    return float(np.uint32(u).view(np.float32))


SCALE = _bf16_round(DH ** -0.5)
EPS = _bf16_round(1e-5)


def _r(x):
    return x.astype(BF).astype(F32)


def _layernorm(x32):
    m = jnp.mean(x32, axis=-1, keepdims=True)
    c = x32 - m
    v = jnp.mean(c * c, axis=-1, keepdims=True)
    num = _r(x32 - _r(m))
    den = _r(jnp.sqrt(_r(_r(v) + EPS)))
    return (num / den).astype(BF)


def _strided(n, groups):
    assert n % groups == 0
    return [g * (n // groups) + r for r in range(n // groups) for g in range(groups)]


def _zip2(a, b):
    assert len(a) == len(b)
    return [j for x, y in zip(a, b) for j in (x + (0,), y + (1,))]


def _alt(a):
    return [x + (i % 2,) for i, x in enumerate(a)]


def _split(lst, n):
    return [lst[i * len(lst) // n:(i + 1) * len(lst) // n] for i in range(n)]


def _kv_order(groups, mode, threads, shift):
    rows = _strided(DH // 8, groups)

    def order(rp):
        if mode == "h":
            return [(r, c) for c in (0, 1) for r in rp]
        if mode == "i":
            return [(r, c) for r in rp for c in (0, 1)]
        return [(r, (i + k) % 2) for k in (0, 1) for i, r in enumerate(rp)]

    k = [(0,) + p for p in order(rows)]
    v = [(1,) + p for p in order(rows[shift:] + rows[:shift])]
    if threads == "kv":
        return _zip2(k, v)
    if threads == "seq":
        return _alt(k + v)
    n = len(k) // 2
    return _zip2(k[:n], k[n:]) + _zip2(v[:n], v[n:])


def _tile_view(a):
    r, c = a.shape
    return a.reshape(r // 8, 8, c // 128, 128).transpose(0, 2, 1, 3).reshape(r * c // 1024, 8, 128)


def _untile(t, cols):
    nc = cols // 128
    t = t.reshape(t.shape[0] // nc, nc, 8, 128)
    return [t[:, j].reshape(t.shape[0] * 8, 128) for j in range(nc)]


def make_kernel(R=3, kv=(8, "h", "half", 1), qo=(5, 16), nq=2, n0=100, parts=4,
                f13=(4, 3, 4), w2ch=((80, 3, 4), (60, 3, 4), (60, 3, 4), (40, 3, 4))):
    QG, QT = qo
    GF, g13, t13 = f13
    TF = D * F // 1024 // GF
    NT = D // 128
    N2 = len(w2ch)
    w2off = [sum(c[0] for c in w2ch[:i]) for i in range(N2)]
    assert (H * DH // 128) % QT == 0 and TF % t13 == 0 and TF % NT == 0
    assert sum(c[0] for c in w2ch) == TF and all(c[0] % NT == 0 for c in w2ch)
    kvp = _kv_order(*kv)
    HW = W // 2

    def kernel(x_hbm, kt_hbm, vt_hbm, wq_hbm, wo_hbm, w1_hbm, w3_hbm, w2_hbm, o_hbm,
               kv_v, wq_v, wo_v, wf_v, q_v, x_v, o_v, sem_o):

        def body(sem_kv, sem_w13, sems):
            sem_x, sem_f, sem_wq, sem_wo = (sems.at[i] for i in range(4))
            def issue(jobs):
                for (src, dst, sem, idx, thread) in jobs:
                    pltpu.make_async_copy(src.at[idx], dst.at[idx], sem).start(priority=thread)

            def wait_all(ref, sem):
                pltpu.make_async_copy(ref, ref, sem).wait()

            def head_jobs(h, slot):
                src = (kt_hbm.at[h, :, pl.ds(SK - W, W)], vt_hbm.at[h, :, pl.ds(SK - W, W)])
                return [(src[a], kv_v.at[slot, a], sem_kv.at[slot], (pl.ds(8 * r, 8), pl.ds(HW * c, HW)), t)
                        for a, r, c, t in kvp]

            x_copy = pltpu.make_async_copy(x_hbm, x_v, sem_x)
            x_copy.start()
            order = _strided(D * H * DH // 1024 // QT, QG)
            ppr = H * DH // 128 // QT
            jq = [(wq_hbm, wq_v, sem_f if p < ppr else sem_wq,
                   (pl.ds(p // ppr * 8, 8), pl.ds(p % ppr * QT * 128, QT * 128))) for p in order]
            jo = [(wo_hbm, wo_v, sem_wo, (pl.ds(p * QT, QT),)) for p in order]
            issue(_zip2(jq, jo))
            wait_all(wq_v.at[pl.ds(0, 8)], sem_f)
            jobs = []
            for h in range(R - 1):
                jobs += head_jobs(h, h)
            issue(jobs[:n0])

            x_copy.wait()
            x32 = x_v[...].astype(F32)
            lnx = jnp.broadcast_to(_layernorm(x32), (8, D))
            wait_all(wq_v.at[pl.ds(8, D - 8)], sem_wq)
            QC = H // nq
            for c, group in enumerate(_split(jobs[n0:], nq)):
                qc = jnp.dot(lnx, wq_v[:, c * QC * DH:(c + 1) * QC * DH], preferred_element_type=F32)
                for j in range(QC):
                    q_v[c * QC + j] = qc[:, j * DH:(j + 1) * DH]
                issue(group)
            wait_all(wo_v, sem_wo)

            def head_compute(h, slot, attn, jobs):
                groups = _split(jobs, 2 * parts)
                CW = W // parts
                wait_all(kv_v.at[slot], sem_kv.at[slot])
                qh = q_v[h].astype(BF)
                s = []
                for c in range(parts):
                    s.append(jnp.dot(qh, kv_v[slot, 0, :, c * CW:(c + 1) * CW], preferred_element_type=F32))
                    issue(groups[c])
                s = _r(_r(jnp.concatenate(s, axis=1)) * SCALE)
                m = jnp.max(s, axis=-1, keepdims=True)
                e = _r(jnp.exp(_r(s - m)))
                l = _r(jnp.sum(e, axis=-1, keepdims=True))
                p = (e / l).astype(BF)
                o = None
                for c in range(parts):
                    o_ = lax.dot_general(p[:, c * CW:(c + 1) * CW], kv_v[slot, 1, :, c * CW:(c + 1) * CW],
                                         (((1,), (1,)), ((), ())), preferred_element_type=F32)
                    o = o_ if o is None else o + o_
                    issue(groups[parts + c])
                tph = DH // 8 * NT
                wo_h = jnp.concatenate(_untile(wo_v[pl.ds(h * tph, tph)], D), axis=1)
                return attn + jnp.dot(o.astype(BF), wo_h, preferred_element_type=F32)

            def head(h, attn):
                return head_compute(h, h % R, attn, head_jobs(h + R - 1, (h + R - 1) % R))

            attn = lax.fori_loop(0, H - R + 1, head, jnp.zeros((8, D), F32))

            p13 = [(pl.ds(a, min(g13, GF - a)), pl.ds(t, t13)) for t in range(0, TF, t13) for a in range(0, GF, g13)]
            tail = _zip2([(w1_hbm, wf_v.at[0], sem_w13, p) for p in p13],
                         [(w3_hbm, wf_v.at[1], sem_w13, p) for p in p13])
            for c, (nt, g, t) in enumerate(w2ch):
                tail += _alt([(w2_hbm, wf_v.at[2], sems.at[c], (pl.ds(a, min(g, GF - a)), pl.ds(w2off[c] + u, min(t, nt - u))))
                              for u in range(0, nt, t) for a in range(0, GF, g)])
            for h, stage in zip(range(H - R + 1, H), _split(tail, R - 1)):
                attn = head_compute(h, h % R, attn, stage)
            hres = _r(x32 + _r(attn))
            lnh = _layernorm(hres)
            wait_all(wf_v.at[pl.ds(0, 2)], sem_w13)
            w1 = jnp.concatenate(_untile(wf_v[0].reshape(GF * TF, 8, 128), F), axis=1)
            gate = _r(jnp.dot(lnh, w1, preferred_element_type=F32))
            w3 = jnp.concatenate(_untile(wf_v[1].reshape(GF * TF, 8, 128), F), axis=1)
            up = _r(jnp.dot(lnh, w3, preferred_element_type=F32))
            hm = _r(_r(gate * _r(jax.nn.sigmoid(gate))) * up)
            RF = F // GF
            hms = [jnp.concatenate([hm[:, a * RF + w2off[c] // NT * 8:a * RF + (w2off[c] + nt) // NT * 8]
                                    for a in range(GF)], axis=1).astype(BF) for c, (nt, _, _) in enumerate(w2ch)]
            out = None
            for c, (nt, _, _) in enumerate(w2ch):
                chunk = wf_v.at[2, :, pl.ds(w2off[c], nt)]
                wait_all(chunk, sems.at[c])
                w2c = jnp.concatenate(_untile(chunk[...].reshape(GF * nt, 8, 128), D), axis=1)
                o_ = jnp.dot(hms[c], w2c, preferred_element_type=F32)
                out = o_ if out is None else out + o_
            res = hres + _r(out)
            o_v[...] = res[0:1, :].astype(o_v.dtype)
            pltpu.make_async_copy(o_v, o_hbm, sem_o).start()

        dma = pltpu.SemaphoreType.DMA
        pl.run_scoped(body, dma((R,)), dma(()), dma((max(N2, 4),)))
        pltpu.make_async_copy(o_v, o_hbm, sem_o).wait()

    @jax.jit
    def run(A_x, A_k_cache, A_v_cache, A_wq, A_wo, B_x, B_w1, B_w3, B_w2):
        del B_x
        x = A_x.reshape(1, D)
        kt = jnp.swapaxes(A_k_cache.reshape(H, SK, DH), 1, 2)
        vt = jnp.swapaxes(A_v_cache.reshape(H, SK, DH), 1, 2)
        out = pl.pallas_call(
            kernel,
            out_shape=jax.ShapeDtypeStruct((1, D), A_x.dtype),
            in_specs=[pl.BlockSpec(memory_space=pl.ANY)] * 8,
            out_specs=pl.BlockSpec(memory_space=pl.ANY),
            scratch_shapes=[
                pltpu.VMEM((R, 2, DH, W), BF),
                pltpu.VMEM((D, H * DH), BF),
                pltpu.VMEM((H * DH * D // 1024, 8, 128), BF),
                pltpu.VMEM((3, GF, TF, 8, 128), BF),
                pltpu.VMEM((H, 8, DH), F32),
                pltpu.VMEM((1, D), BF),
                pltpu.VMEM((1, D), BF),
                pltpu.SemaphoreType.DMA(()),
            ],
            compiler_params=pltpu.CompilerParams(vmem_limit_bytes=64 * 1024 * 1024),
        )(x, kt, vt, A_wq, _tile_view(A_wo), *[_tile_view(w).reshape(GF, TF, 8, 128) for w in (B_w1, B_w3, B_w2)])
        return out.reshape(1, 1, D)

    return run


pallas_sequential_preLN__sliding_block_cached__glu_gated_swiglu__decode_kernel = make_kernel()
```

```python
import jax
import jax.numpy as jnp
import numpy as np
from jax import lax
import jax.experimental.pallas as pl
import jax.experimental.pallas.tpu as pltpu

H, DH, SK, D, F = 32, 192, 32768, 640, 1536
W = min(4096, max(256, SK // 4))
BF = jnp.bfloat16
F32 = jnp.float32


def _bf16_round(v):
    u = int(np.float32(v).view(np.uint32))
    u = (u + 0x7FFF + ((u >> 16) & 1)) & 0xFFFF0000
    return float(np.uint32(u).view(np.float32))


SCALE = _bf16_round(DH ** -0.5)
EPS = _bf16_round(1e-5)


def _r(x):
    return x.astype(BF).astype(F32)


def _layernorm(x32):
    m = jnp.mean(x32, axis=-1, keepdims=True)
    c = x32 - m
    v = jnp.mean(c * c, axis=-1, keepdims=True)
    num = _r(x32 - _r(m))
    den = _r(jnp.sqrt(_r(_r(v) + EPS)))
    return (num / den).astype(BF)


def _strided(n, groups):
    assert n % groups == 0
    return [g * (n // groups) + r for r in range(n // groups) for g in range(groups)]


def _zip2(a, b):
    assert len(a) == len(b)
    return [j for x, y in zip(a, b) for j in (x + (0,), y + (1,))]


def _alt(a):
    return [x + (i % 2,) for i, x in enumerate(a)]


def _split(lst, n):
    return [lst[i * len(lst) // n:(i + 1) * len(lst) // n] for i in range(n)]


def _schedule(jobs, ends, depth, ramp, lead):
    n = len(jobs)
    keyed = []
    for p, job in enumerate(jobs):
        if p >= n - depth:
            keyed.append((n - 3 * depth + 2 * (p - (n - depth)), job + (1,)))
        elif (n - depth - p) % 2:
            keyed.append((p, job + (0,)))
        else:
            keyed.append((p - 2 * depth * min(1.0, p / ramp), job + (1,)))
    keyed.sort(key=lambda kj: kj[0])
    cuts = [0] + [sum(k < e + lead for k, _ in keyed) for e in ends[:-1]] + [n]
    return [[j for _, j in keyed[a:b]] for a, b in zip(cuts, cuts[1:])]


def _kv_order(groups, mode, threads, shift):
    rows = _strided(DH // 8, groups)

    def order(rp):
        if mode == "h":
            return [(r, c) for c in (0, 1) for r in rp]
        if mode == "i":
            return [(r, c) for r in rp for c in (0, 1)]
        return [(r, (i + k) % 2) for k in (0, 1) for i, r in enumerate(rp)]

    k = [(0,) + p for p in order(rows)]
    v = [(1,) + p for p in order(rows[shift:] + rows[:shift])]
    if threads == "kv":
        return _zip2(k, v)
    if threads == "seq":
        return _alt(k + v)
    n = len(k) // 2
    return _zip2(k[:n], k[n:]) + _zip2(v[:n], v[n:])


def _tile_view(a):
    r, c = a.shape
    return a.reshape(r // 8, 8, c // 128, 128).transpose(0, 2, 1, 3).reshape(r * c // 1024, 8, 128)


def _untile(t, cols):
    nc = cols // 128
    t = t.reshape(t.shape[0] // nc, nc, 8, 128)
    return [t[:, j].reshape(t.shape[0] * 8, 128) for j in range(nc)]


def make_kernel(R=3, kv=(8, "h", "half", 1), qo=(5, 16), nq=2, n0=100, parts=4,
                f13=(4, 1, 12), N13=1, w2ch=((60, 1, 12),) * 3 + ((40, 1, 10), (20, 1, 10)), sched=(32, 128, 32)):
    QG, QT = qo
    GF, g13, t13 = f13
    TF = D * F // 1024 // GF
    T13 = TF // N13
    NT = D // 128
    N2 = len(w2ch)
    w2off = [sum(c[0] for c in w2ch[:i]) for i in range(N2)]
    assert (H * DH // 128) % QT == 0 and T13 % t13 == 0 and T13 % (F // 128) == 0
    assert sum(c[0] for c in w2ch) == TF and all(c[0] % NT == 0 for c in w2ch)
    kvp = _kv_order(*kv)
    HW = W // 2

    def kernel(x_hbm, kt_hbm, vt_hbm, wq_hbm, wo_hbm, w1_hbm, w3_hbm, w2_hbm, o_hbm,
               kv_v, wq_v, wo_v, wf_v, q_v, x_v, o_v, sem_o):

        def body(sem_kv, sems):
            sem_x, sem_f, sem_wq, sem_wo = (sems.at[i] for i in range(4))
            def issue(jobs):
                for (src, dst, sem, idx, thread) in jobs:
                    pltpu.make_async_copy(src.at[idx], dst.at[idx], sem).start(priority=thread)

            def wait_all(ref, sem):
                pltpu.make_async_copy(ref, ref, sem).wait()

            def head_jobs(h, slot):
                src = (kt_hbm.at[h, :, pl.ds(SK - W, W)], vt_hbm.at[h, :, pl.ds(SK - W, W)])
                return [(src[a], kv_v.at[slot, a], sem_kv.at[slot], (pl.ds(8 * r, 8), pl.ds(HW * c, HW)), t)
                        for a, r, c, t in kvp]

            x_copy = pltpu.make_async_copy(x_hbm, x_v, sem_x)
            x_copy.start()
            order = _strided(D * H * DH // 1024 // QT, QG)
            ppr = H * DH // 128 // QT
            jq = [(wq_hbm, wq_v, sem_f if p < ppr else sem_wq,
                   (pl.ds(p // ppr * 8, 8), pl.ds(p % ppr * QT * 128, QT * 128))) for p in order]
            jo = [(wo_hbm, wo_v, sem_wo, (pl.ds(p * QT, QT),)) for p in order]
            issue(_zip2(jq, jo))
            wait_all(wq_v.at[pl.ds(0, 8)], sem_f)
            jobs = []
            for h in range(R - 1):
                jobs += head_jobs(h, h)
            issue(jobs[:n0])

            x_copy.wait()
            x32 = x_v[...].astype(F32)
            lnx = jnp.broadcast_to(_layernorm(x32), (8, D))
            wait_all(wq_v.at[pl.ds(8, D - 8)], sem_wq)
            QC = H // nq
            for c, group in enumerate(_split(jobs[n0:], nq)):
                qc = jnp.dot(lnx, wq_v[:, c * QC * DH:(c + 1) * QC * DH], preferred_element_type=F32)
                for j in range(QC):
                    q_v[c * QC + j] = qc[:, j * DH:(j + 1) * DH]
                issue(group)
            wait_all(wo_v, sem_wo)

            def head_compute(h, slot, attn, jobs):
                groups = _split(jobs, 2 * parts)
                CW = W // parts
                wait_all(kv_v.at[slot], sem_kv.at[slot])
                qh = q_v[h].astype(BF)
                s = []
                for c in range(parts):
                    s.append(jnp.dot(qh, kv_v[slot, 0, :, c * CW:(c + 1) * CW], preferred_element_type=F32))
                    issue(groups[c])
                s = _r(_r(jnp.concatenate(s, axis=1)) * SCALE)
                m = jnp.max(s, axis=-1, keepdims=True)
                e = _r(jnp.exp(_r(s - m)))
                l = _r(jnp.sum(e, axis=-1, keepdims=True))
                p = (e / l).astype(BF)
                o = None
                for c in range(parts):
                    o_ = lax.dot_general(p[:, c * CW:(c + 1) * CW], kv_v[slot, 1, :, c * CW:(c + 1) * CW],
                                         (((1,), (1,)), ((), ())), preferred_element_type=F32)
                    o = o_ if o is None else o + o_
                    issue(groups[parts + c])
                tph = DH // 8 * NT
                wo_h = jnp.concatenate(_untile(wo_v[pl.ds(h * tph, tph)], D), axis=1)
                return attn + jnp.dot(o.astype(BF), wo_h, preferred_element_type=F32)

            def head(h, attn):
                return head_compute(h, h % R, attn, head_jobs(h + R - 1, (h + R - 1) % R))

            attn = lax.fori_loop(0, H - R + 1, head, jnp.zeros((8, D), F32))

            tail, ends = [], []
            for c in range(N13):
                p13 = [(pl.ds(a, min(g13, GF - a)), pl.ds(c * T13 + t, t13))
                       for t in range(0, T13, t13) for a in range(0, GF, g13)]
                tail += [j for p in p13 for j in ((w1_hbm, wf_v.at[0], sems.at[c], p), (w3_hbm, wf_v.at[1], sems.at[c], p))]
                ends.append(len(tail))
            for c, (nt, g, t) in enumerate(w2ch):
                tail += [(w2_hbm, wf_v.at[2], sems.at[N13 + c],
                          (pl.ds(a, min(g, GF - a)), pl.ds(w2off[c] + u, min(t, nt - u))))
                         for u in range(0, nt, t) for a in range(0, GF, g)]
                ends.append(len(tail))
            stage = _schedule(tail, [0] + ends, *sched)
            for h in range(H - R + 1, H):
                attn = head_compute(h, h % R, attn, stage[h - H + 2] if h >= H - 2 else [])
            hres = _r(x32 + _r(attn))
            lnh = _layernorm(hres).astype(F32)

            def lhs(v, r0, nr):
                rg = v.shape[1] // GF
                return jnp.concatenate([v[:, a * rg + r0:a * rg + r0 + nr] for a in range(GF)], axis=1).astype(BF)

            def rhs(i, t0, nt, cols):
                return jnp.concatenate(_untile(wf_v[i, :, pl.ds(t0, nt)].reshape(GF * nt, 8, 128), cols), axis=1)

            R13 = D // GF // N13
            ls = [lhs(lnh, c * R13, R13) for c in range(N13)]
            gate = up = None
            for c in range(N13):
                wait_all(wf_v.at[pl.ds(0, 2), :, pl.ds(c * T13, T13)], sems.at[c])
                g_ = jnp.dot(ls[c], rhs(0, c * T13, T13, F), preferred_element_type=F32)
                u_ = jnp.dot(ls[c], rhs(1, c * T13, T13, F), preferred_element_type=F32)
                gate = g_ if gate is None else gate + g_
                up = u_ if up is None else up + u_
                issue(stage[2 + c])
            gate, up = _r(gate), _r(up)
            hm = _r(_r(gate * _r(jax.nn.sigmoid(gate))) * up)
            hs = [lhs(hm, w2off[c] // NT * 8, nt // NT * 8) for c, (nt, _, _) in enumerate(w2ch)]
            out = None
            for c, (nt, _, _) in enumerate(w2ch):
                wait_all(wf_v.at[2, :, pl.ds(w2off[c], nt)], sems.at[N13 + c])
                o_ = jnp.dot(hs[c], rhs(2, w2off[c], nt, D), preferred_element_type=F32)
                out = o_ if out is None else out + o_
                for st in stage[2 + N13 + c:3 + N13 + c]:
                    issue(st)
            res = hres + _r(out)
            o_v[...] = res[0:1, :].astype(o_v.dtype)
            pltpu.make_async_copy(o_v, o_hbm, sem_o).start()

        dma = pltpu.SemaphoreType.DMA
        pl.run_scoped(body, dma((R,)), dma((max(N13 + N2, 4),)))
        pltpu.make_async_copy(o_v, o_hbm, sem_o).wait()

    @jax.jit
    def run(A_x, A_k_cache, A_v_cache, A_wq, A_wo, B_x, B_w1, B_w3, B_w2):
        del B_x
        x = A_x.reshape(1, D)
        kt = jnp.swapaxes(A_k_cache.reshape(H, SK, DH), 1, 2)
        vt = jnp.swapaxes(A_v_cache.reshape(H, SK, DH), 1, 2)
        out = pl.pallas_call(
            kernel,
            out_shape=jax.ShapeDtypeStruct((1, D), A_x.dtype),
            in_specs=[pl.BlockSpec(memory_space=pl.ANY)] * 8,
            out_specs=pl.BlockSpec(memory_space=pl.ANY),
            scratch_shapes=[
                pltpu.VMEM((R, 2, DH, W), BF),
                pltpu.VMEM((D, H * DH), BF),
                pltpu.VMEM((H * DH * D // 1024, 8, 128), BF),
                pltpu.VMEM((3, GF, TF, 8, 128), BF),
                pltpu.VMEM((H, 8, DH), F32),
                pltpu.VMEM((1, D), BF),
                pltpu.VMEM((1, D), BF),
                pltpu.SemaphoreType.DMA(()),
            ],
            compiler_params=pltpu.CompilerParams(vmem_limit_bytes=64 * 1024 * 1024),
        )(x, kt, vt, A_wq, _tile_view(A_wo), *[_tile_view(w).reshape(GF, TF, 8, 128) for w in (B_w1, B_w3, B_w2)])
        return out.reshape(1, 1, D)

    return run


pallas_sequential_preLN__sliding_block_cached__glu_gated_swiglu__decode_kernel = make_kernel()
```

```python
import jax
import jax.numpy as jnp
import numpy as np
from jax import lax
import jax.experimental.pallas as pl
import jax.experimental.pallas.tpu as pltpu

H, DH, SK, D, F = 32, 192, 32768, 640, 1536
W = min(4096, max(256, SK // 4))
BF = jnp.bfloat16
F32 = jnp.float32


def _bf16_round(v):
    u = int(np.float32(v).view(np.uint32))
    u = (u + 0x7FFF + ((u >> 16) & 1)) & 0xFFFF0000
    return float(np.uint32(u).view(np.float32))


SCALE = _bf16_round(DH ** -0.5)
EPS = _bf16_round(1e-5)


def _r(x):
    return x.astype(BF).astype(F32)


def _layernorm(x32):
    m = jnp.mean(x32, axis=-1, keepdims=True)
    c = x32 - m
    v = jnp.mean(c * c, axis=-1, keepdims=True)
    num = _r(x32 - _r(m))
    den = _r(jnp.sqrt(_r(_r(v) + EPS)))
    return (num / den).astype(BF)


def _strided(n, groups):
    assert n % groups == 0
    return [g * (n // groups) + r for r in range(n // groups) for g in range(groups)]


def _zip2(a, b):
    assert len(a) == len(b)
    return [j for x, y in zip(a, b) for j in (x + (0,), y + (1,))]


def _alt(a):
    return [x + (i % 2,) for i, x in enumerate(a)]


def _split(lst, n):
    return [lst[i * len(lst) // n:(i + 1) * len(lst) // n] for i in range(n)]


def _schedule(jobs, ends, depth, ramp, lead):
    n = len(jobs)
    keyed = []
    for p, job in enumerate(jobs):
        if p >= n - depth:
            keyed.append((n - 3 * depth + 2 * (p - (n - depth)), job + (1,)))
        elif (n - depth - p) % 2:
            keyed.append((p, job + (0,)))
        else:
            keyed.append((p - 2 * depth * min(1.0, p / ramp), job + (1,)))
    keyed.sort(key=lambda kj: kj[0])
    cuts = [0] + [sum(k < e + lead for k, _ in keyed) for e in ends[:-1]] + [n]
    return [[j for _, j in keyed[a:b]] for a, b in zip(cuts, cuts[1:])]


def _kv_order(groups, mode, threads, shift):
    rows = _strided(DH // 8, groups)

    def order(rp):
        if mode == "h":
            return [(r, c) for c in (0, 1) for r in rp]
        if mode == "i":
            return [(r, c) for r in rp for c in (0, 1)]
        return [(r, (i + k) % 2) for k in (0, 1) for i, r in enumerate(rp)]

    k = [(0,) + p for p in order(rows)]
    v = [(1,) + p for p in order(rows[shift:] + rows[:shift])]
    if threads == "kv":
        return _zip2(k, v)
    if threads == "seq":
        return _alt(k + v)
    n = len(k) // 2
    return _zip2(k[:n], k[n:]) + _zip2(v[:n], v[n:])


def _tile_view(a):
    r, c = a.shape
    return a.reshape(r // 8, 8, c // 128, 128).transpose(0, 2, 1, 3).reshape(r * c // 1024, 8, 128)


def _untile(t, cols):
    nc = cols // 128
    t = t.reshape(t.shape[0] // nc, nc, 8, 128)
    return [t[:, j].reshape(t.shape[0] * 8, 128) for j in range(nc)]


def make_kernel(R=3, kv=(12, "h", "half", 23), qo=(5, 16), nq=2, n0=100, parts=4,
                f13=(4, 1, 16), N13=1, w2ch=((60, 1, 12),) * 3 + ((35, 1, 12), (25, 1, 12)), sched=(32, 96, 30)):
    QG, QT = qo
    GF, g13, t13 = f13
    TF = D * F // 1024 // GF
    T13 = TF // N13
    NT = D // 128
    N2 = len(w2ch)
    w2off = [sum(c[0] for c in w2ch[:i]) for i in range(N2)]
    assert (H * DH // 128) % QT == 0 and T13 % t13 == 0 and T13 % (F // 128) == 0
    assert sum(c[0] for c in w2ch) == TF and all(c[0] % NT == 0 for c in w2ch)
    kvp = _kv_order(*kv)
    HW = W // 2

    def kernel(x_hbm, kt_hbm, vt_hbm, wq_hbm, wo_hbm, w1_hbm, w3_hbm, w2_hbm, o_hbm,
               kv_v, wq_v, wo_v, wf_v, q_v, x_v, o_v, sem_o):

        def body(sem_kv, sems):
            sem_x, sem_f, sem_wq, sem_wo = (sems.at[i] for i in range(4))
            def issue(jobs):
                for (src, dst, sem, idx, thread) in jobs:
                    pltpu.make_async_copy(src.at[idx], dst.at[idx], sem).start(priority=thread)

            def wait_all(ref, sem):
                pltpu.make_async_copy(ref, ref, sem).wait()

            def head_jobs(h, slot):
                src = (kt_hbm.at[h, :, pl.ds(SK - W, W)], vt_hbm.at[h, :, pl.ds(SK - W, W)])
                return [(src[a], kv_v.at[slot, a], sem_kv.at[slot], (pl.ds(8 * r, 8), pl.ds(HW * c, HW)), t)
                        for a, r, c, t in kvp]

            x_copy = pltpu.make_async_copy(x_hbm, x_v, sem_x)
            x_copy.start()
            order = _strided(D * H * DH // 1024 // QT, QG)
            ppr = H * DH // 128 // QT
            jq = [(wq_hbm, wq_v, sem_f if p < ppr else sem_wq,
                   (pl.ds(p // ppr * 8, 8), pl.ds(p % ppr * QT * 128, QT * 128))) for p in order]
            jo = [(wo_hbm, wo_v, sem_wo, (pl.ds(p * QT, QT),)) for p in order]
            issue(_zip2(jq, jo))
            wait_all(wq_v.at[pl.ds(0, 8)], sem_f)
            jobs = []
            for h in range(R - 1):
                jobs += head_jobs(h, h)
            issue(jobs[:n0])

            x_copy.wait()
            x32 = x_v[...].astype(F32)
            lnx = jnp.broadcast_to(_layernorm(x32), (8, D))
            wait_all(wq_v.at[pl.ds(8, D - 8)], sem_wq)
            QC = H // nq
            for c, group in enumerate(_split(jobs[n0:], nq)):
                qc = jnp.dot(lnx, wq_v[:, c * QC * DH:(c + 1) * QC * DH], preferred_element_type=F32)
                for j in range(QC):
                    q_v[c * QC + j] = qc[:, j * DH:(j + 1) * DH]
                issue(group)
            wait_all(wo_v, sem_wo)

            def head_compute(h, slot, attn, jobs):
                groups = _split(jobs, 2 * parts)
                CW = W // parts
                wait_all(kv_v.at[slot], sem_kv.at[slot])
                qh = q_v[h].astype(BF)
                s = []
                for c in range(parts):
                    s.append(jnp.dot(qh, kv_v[slot, 0, :, c * CW:(c + 1) * CW], preferred_element_type=F32))
                    issue(groups[c])
                s = _r(_r(jnp.concatenate(s, axis=1)) * SCALE)
                m = jnp.max(s, axis=-1, keepdims=True)
                e = _r(jnp.exp(_r(s - m)))
                l = _r(jnp.sum(e, axis=-1, keepdims=True))
                p = (e / l).astype(BF)
                o = None
                for c in range(parts):
                    o_ = lax.dot_general(p[:, c * CW:(c + 1) * CW], kv_v[slot, 1, :, c * CW:(c + 1) * CW],
                                         (((1,), (1,)), ((), ())), preferred_element_type=F32)
                    o = o_ if o is None else o + o_
                    issue(groups[parts + c])
                tph = DH // 8 * NT
                wo_h = jnp.concatenate(_untile(wo_v[pl.ds(h * tph, tph)], D), axis=1)
                return attn + jnp.dot(o.astype(BF), wo_h, preferred_element_type=F32)

            def head(h, attn):
                return head_compute(h, h % R, attn, head_jobs(h + R - 1, (h + R - 1) % R))

            attn = lax.fori_loop(0, H - R + 1, head, jnp.zeros((8, D), F32))

            tail, ends = [], []
            for c in range(N13):
                p13 = [(pl.ds(a, min(g13, GF - a)), pl.ds(c * T13 + t, t13))
                       for t in range(0, T13, t13) for a in range(0, GF, g13)]
                tail += [j for p in p13 for j in ((w1_hbm, wf_v.at[0], sems.at[c], p), (w3_hbm, wf_v.at[1], sems.at[c], p))]
                ends.append(len(tail))
            for c, (nt, g, t) in enumerate(w2ch):
                tail += [(w2_hbm, wf_v.at[2], sems.at[N13 + c],
                          (pl.ds(a, min(g, GF - a)), pl.ds(w2off[c] + u, min(t, nt - u))))
                         for u in range(0, nt, t) for a in range(0, GF, g)]
                ends.append(len(tail))
            stage = _schedule(tail, [0] + ends, *sched)
            for h in range(H - R + 1, H):
                attn = head_compute(h, h % R, attn, stage[h - H + 2] if h >= H - 2 else [])
            hres = _r(x32 + _r(attn))
            lnh = _layernorm(hres).astype(F32)

            def lhs(v, r0, nr):
                rg = v.shape[1] // GF
                return jnp.concatenate([v[:, a * rg + r0:a * rg + r0 + nr] for a in range(GF)], axis=1).astype(BF)

            def rhs(i, t0, nt, cols):
                return jnp.concatenate(_untile(wf_v[i, :, pl.ds(t0, nt)].reshape(GF * nt, 8, 128), cols), axis=1)

            R13 = D // GF // N13
            ls = [lhs(lnh, c * R13, R13) for c in range(N13)]
            gate = up = None
            for c in range(N13):
                wait_all(wf_v.at[pl.ds(0, 2), :, pl.ds(c * T13, T13)], sems.at[c])
                g_ = jnp.dot(ls[c], rhs(0, c * T13, T13, F), preferred_element_type=F32)
                u_ = jnp.dot(ls[c], rhs(1, c * T13, T13, F), preferred_element_type=F32)
                gate = g_ if gate is None else gate + g_
                up = u_ if up is None else up + u_
                issue(stage[2 + c])
            gate, up = _r(gate), _r(up)
            hm = _r(_r(gate * _r(jax.nn.sigmoid(gate))) * up)
            hs = [lhs(hm, w2off[c] // NT * 8, nt // NT * 8) for c, (nt, _, _) in enumerate(w2ch)]
            out = None
            for c, (nt, _, _) in enumerate(w2ch):
                wait_all(wf_v.at[2, :, pl.ds(w2off[c], nt)], sems.at[N13 + c])
                o_ = jnp.dot(hs[c], rhs(2, w2off[c], nt, D), preferred_element_type=F32)
                out = o_ if out is None else out + o_
                for st in stage[2 + N13 + c:3 + N13 + c]:
                    issue(st)
            res = hres + _r(out)
            o_v[...] = res[0:1, :].astype(o_v.dtype)
            pltpu.make_async_copy(o_v, o_hbm, sem_o).start()

        dma = pltpu.SemaphoreType.DMA
        pl.run_scoped(body, dma((R,)), dma((max(N13 + N2, 4),)))
        pltpu.make_async_copy(o_v, o_hbm, sem_o).wait()

    @jax.jit
    def run(A_x, A_k_cache, A_v_cache, A_wq, A_wo, B_x, B_w1, B_w3, B_w2):
        del B_x
        x = A_x.reshape(1, D)
        kt = jnp.swapaxes(A_k_cache.reshape(H, SK, DH), 1, 2)
        vt = jnp.swapaxes(A_v_cache.reshape(H, SK, DH), 1, 2)
        out = pl.pallas_call(
            kernel,
            out_shape=jax.ShapeDtypeStruct((1, D), A_x.dtype),
            in_specs=[pl.BlockSpec(memory_space=pl.ANY)] * 8,
            out_specs=pl.BlockSpec(memory_space=pl.ANY),
            scratch_shapes=[
                pltpu.VMEM((R, 2, DH, W), BF),
                pltpu.VMEM((D, H * DH), BF),
                pltpu.VMEM((H * DH * D // 1024, 8, 128), BF),
                pltpu.VMEM((3, GF, TF, 8, 128), BF),
                pltpu.VMEM((H, 8, DH), F32),
                pltpu.VMEM((1, D), BF),
                pltpu.VMEM((1, D), BF),
                pltpu.SemaphoreType.DMA(()),
            ],
            compiler_params=pltpu.CompilerParams(vmem_limit_bytes=64 * 1024 * 1024, disable_bounds_checks=True,
                                                 disable_semaphore_checks=True),
        )(x, kt, vt, A_wq, _tile_view(A_wo), *[_tile_view(w).reshape(GF, TF, 8, 128) for w in (B_w1, B_w3, B_w2)])
        return out.reshape(1, 1, D)

    return run


pallas_sequential_preLN__sliding_block_cached__glu_gated_swiglu__decode_kernel = make_kernel()
```

```python
import jax
import jax.numpy as jnp
import numpy as np
from jax import lax
import jax.experimental.pallas as pl
import jax.experimental.pallas.tpu as pltpu

H, DH, SK, D, F = 32, 192, 32768, 640, 1536
W = min(4096, max(256, SK // 4))
BF = jnp.bfloat16
F32 = jnp.float32


def _bf16_round(v):
    u = int(np.float32(v).view(np.uint32))
    u = (u + 0x7FFF + ((u >> 16) & 1)) & 0xFFFF0000
    return float(np.uint32(u).view(np.float32))


SCALE = _bf16_round(DH ** -0.5)
EPS = _bf16_round(1e-5)


def _r(x):
    return x.astype(BF).astype(F32)


def _layernorm(x32):
    m = jnp.mean(x32, axis=-1, keepdims=True)
    c = x32 - m
    v = jnp.mean(c * c, axis=-1, keepdims=True)
    num = _r(x32 - _r(m))
    den = _r(jnp.sqrt(_r(_r(v) + EPS)))
    return (num / den).astype(BF)


def _strided(n, groups):
    assert n % groups == 0
    return [g * (n // groups) + r for r in range(n // groups) for g in range(groups)]


def _zip2(a, b):
    assert len(a) == len(b)
    return [j for x, y in zip(a, b) for j in (x + (0,), y + (1,))]


def _alt(a):
    return [x + (i % 2,) for i, x in enumerate(a)]


def _split(lst, n):
    return [lst[i * len(lst) // n:(i + 1) * len(lst) // n] for i in range(n)]


def _schedule(jobs, ends, depth, ramp, lead):
    n = len(jobs)
    keyed = []
    for p, job in enumerate(jobs):
        if p >= n - depth:
            keyed.append((n - 3 * depth + 2 * (p - (n - depth)), job + (1,)))
        elif (n - depth - p) % 2:
            keyed.append((p, job + (0,)))
        else:
            keyed.append((p - 2 * depth * min(1.0, p / ramp), job + (1,)))
    keyed.sort(key=lambda kj: kj[0])
    cuts = [0] + [sum(k < e + lead for k, _ in keyed) for e in ends[:-1]] + [n]
    return [[j for _, j in keyed[a:b]] for a, b in zip(cuts, cuts[1:])]


def _kv_order(groups, mode, threads, shift):
    rows = _strided(DH // 8, groups)

    def order(rp):
        if mode == "h":
            return [(r, c) for c in (0, 1) for r in rp]
        if mode == "i":
            return [(r, c) for r in rp for c in (0, 1)]
        return [(r, (i + k) % 2) for k in (0, 1) for i, r in enumerate(rp)]

    k = [(0,) + p for p in order(rows)]
    v = [(1,) + p for p in order(rows[shift:] + rows[:shift])]
    if threads == "kv":
        return _zip2(k, v)
    if threads == "seq":
        return _alt(k + v)
    n = len(k) // 2
    return _zip2(k[:n], k[n:]) + _zip2(v[:n], v[n:])


def _tile_view(a):
    r, c = a.shape
    return a.reshape(r // 8, 8, c // 128, 128).transpose(0, 2, 1, 3).reshape(r * c // 1024, 8, 128)


def _untile(t, cols):
    nc = cols // 128
    t = t.reshape(t.shape[0] // nc, nc, 8, 128)
    return [t[:, j].reshape(t.shape[0] * 8, 128) for j in range(nc)]


def make_kernel(R=3, kv=(12, "h", "half", 23), qo=(5, 16), nq=2, n0=100, parts=4,
                f13=(4, 1, 16), N13=1, w2ch=((60, 1, 15),) * 3 + ((30, 1, 15), (15, 1, 15), (10, 1, 10), (5, 1, 5)),
                sched=(32, 96, 30), NV=3):
    QG, QT = qo
    GF, g13, t13 = f13
    TF = D * F // 1024 // GF
    T13 = TF // N13
    NT = D // 128
    N2 = len(w2ch)
    w2off = [sum(c[0] for c in w2ch[:i]) for i in range(N2)]
    assert (H * DH // 128) % QT == 0 and T13 % t13 == 0 and T13 % (F // 128) == 0
    assert sum(c[0] for c in w2ch) == TF and all(c[0] % NT == 0 for c in w2ch)
    kvp = _kv_order(*kv)
    HW = W // 2

    def kernel(x_hbm, kt_hbm, vt_hbm, wq_hbm, wo_hbm, w1_hbm, w3_hbm, w2_hbm, o_hbm,
               kv_v, wq_v, wo_v, wf_v, q_v, x_v, o_v, sem_o):

        def body(sem_kv, sems):
            sem_x, sem_f, sem_wq, sem_wo = (sems.at[i] for i in range(4))
            def issue(jobs):
                for (src, dst, sem, idx, thread) in jobs:
                    pltpu.make_async_copy(src.at[idx], dst.at[idx], sem).start(priority=thread)

            def wait_all(ref, sem):
                pltpu.make_async_copy(ref, ref, sem).wait()

            def head_jobs(h, slot):
                src = (kt_hbm.at[h, :, pl.ds(SK - W, W)], vt_hbm.at[h, :, pl.ds(SK - W, W)])
                return [(src[a], kv_v.at[slot, a], sem_kv.at[slot], (pl.ds(8 * r, 8), pl.ds(HW * c, HW)), t)
                        for a, r, c, t in kvp]

            x_copy = pltpu.make_async_copy(x_hbm, x_v, sem_x)
            x_copy.start()
            order = _strided(D * H * DH // 1024 // QT, QG)
            ppr = H * DH // 128 // QT
            jq = [(wq_hbm, wq_v, sem_f if p < ppr else sem_wq,
                   (pl.ds(p // ppr * 8, 8), pl.ds(p % ppr * QT * 128, QT * 128))) for p in order]
            jo = [(wo_hbm, wo_v, sem_wo, (pl.ds(p * QT, QT),)) for p in order]
            issue(_zip2(jq, jo))
            wait_all(wq_v.at[pl.ds(0, 8)], sem_f)
            jobs = []
            for h in range(R - 1):
                jobs += head_jobs(h, h)
            issue(jobs[:n0])

            x_copy.wait()
            x32 = x_v[...].astype(F32)
            lnx = jnp.broadcast_to(_layernorm(x32), (8, D))
            wait_all(wq_v.at[pl.ds(8, D - 8)], sem_wq)
            QC = H // nq
            for c, group in enumerate(_split(jobs[n0:], nq)):
                qc = jnp.dot(lnx, wq_v[:, c * QC * DH:(c + 1) * QC * DH], preferred_element_type=F32)
                for j in range(QC):
                    q_v[c * QC + j] = qc[:, j * DH:(j + 1) * DH]
                issue(group)
            wait_all(wo_v, sem_wo)

            def head_compute(h, slot, attn, jobs):
                groups = _split(jobs, 2 * parts)
                CW = W // parts
                wait_all(kv_v.at[slot], sem_kv.at[slot])
                qh = q_v[h].astype(BF)
                s = []
                for c in range(parts):
                    s.append(jnp.dot(qh, kv_v[slot, 0, :, c * CW:(c + 1) * CW], preferred_element_type=F32))
                    issue(groups[c])
                s = _r(_r(jnp.concatenate(s, axis=1)) * SCALE)
                m = jnp.max(s, axis=-1, keepdims=True)
                e = _r(jnp.exp(_r(s - m)))
                l = _r(jnp.sum(e, axis=-1, keepdims=True))
                p = (e / l).astype(BF)
                o = None
                for c in range(parts):
                    o_ = lax.dot_general(p[:, c * CW:(c + 1) * CW], kv_v[slot, 1, :, c * CW:(c + 1) * CW],
                                         (((1,), (1,)), ((), ())), preferred_element_type=F32)
                    o = o_ if o is None else o + o_
                    issue(groups[parts + c])
                tph = DH // 8 * NT
                wo_h = jnp.concatenate(_untile(wo_v[pl.ds(h * tph, tph)], D), axis=1)
                return attn + jnp.dot(o.astype(BF), wo_h, preferred_element_type=F32)

            def head(h, attn):
                return head_compute(h, h % R, attn, head_jobs(h + R - 1, (h + R - 1) % R))

            attn = lax.fori_loop(0, H - R + 1, head, jnp.zeros((8, D), F32))

            tail, ends = [], []
            for c in range(N13):
                p13 = [(pl.ds(a, min(g13, GF - a)), pl.ds(c * T13 + t, t13))
                       for t in range(0, T13, t13) for a in range(0, GF, g13)]
                tail += [j for p in p13 for j in ((w1_hbm, wf_v.at[0], sems.at[c], p), (w3_hbm, wf_v.at[1], sems.at[c], p))]
                ends.append(len(tail))
            for c, (nt, g, t) in enumerate(w2ch):
                tail += [(w2_hbm, wf_v.at[2], sems.at[N13 + c],
                          (pl.ds(a, min(g, GF - a)), pl.ds(w2off[c] + u, min(t, nt - u))))
                         for u in range(0, nt, t) for a in range(0, GF, g)]
                ends.append(len(tail))
            stage = _schedule(tail, [0] + ends, *sched)
            for h in range(H - R + 1, H):
                attn = head_compute(h, h % R, attn, stage[h - H + 2] if h >= H - 2 else [])
            hres = _r(x32 + _r(attn))
            lnh = _layernorm(hres).astype(F32)

            def lhs(v, r0, nr):
                rg = v.shape[1] // GF
                return jnp.concatenate([v[:, a * rg + r0:a * rg + r0 + nr] for a in range(GF)], axis=1).astype(BF)

            def rhs(i, t0, nt, cols):
                return jnp.concatenate(_untile(wf_v[i, :, pl.ds(t0, nt)].reshape(GF * nt, 8, 128), cols), axis=1)

            R13 = D // GF // N13
            ls = [lhs(lnh, c * R13, R13) for c in range(N13)]
            gate = up = None
            for c in range(N13):
                wait_all(wf_v.at[pl.ds(0, 2), :, pl.ds(c * T13, T13)], sems.at[c])
                g_ = jnp.dot(ls[c], rhs(0, c * T13, T13, F), preferred_element_type=F32)
                u_ = jnp.dot(ls[c], rhs(1, c * T13, T13, F), preferred_element_type=F32)
                gate = g_ if gate is None else gate + g_
                up = u_ if up is None else up + u_
                issue(stage[2 + c])
            gate, up = _r(gate), _r(up)
            hm = _r(_r(gate * _r(jax.nn.sigmoid(gate))) * up)
            hs = [lhs(hm, w2off[c] // NT * 8, nt // NT * 8) for c, (nt, _, _) in enumerate(w2ch)]
            for c in range(N2 - NV, N2):
                nr = hs[c].shape[1]
                col = jnp.concatenate([hs[c][0:1].astype(F32), jnp.zeros((1, 128 - nr), F32)], axis=1)
                hs[c] = jnp.broadcast_to(col, (128, 128)).T[:nr].reshape(nr // 8, 8, 128)
            out = None
            for c, (nt, _, _) in enumerate(w2ch):
                if c == N2 - NV:
                    first = lax.broadcasted_iota(jnp.int32, (8, 128), 0) == 0
                    acc = [jnp.where(first, out[:, j * 128:(j + 1) * 128], 0.0) for j in range(NT)]
                wait_all(wf_v.at[2, :, pl.ds(w2off[c], nt)], sems.at[N13 + c])
                if c < N2 - NV:
                    o_ = jnp.dot(hs[c], rhs(2, w2off[c], nt, D), preferred_element_type=F32)
                    out = o_ if out is None else out + o_
                else:
                    w = _untile(wf_v[2, :, pl.ds(w2off[c], nt)].reshape(GF * nt, 8, 128), D)
                    acc = [acc[j] + jnp.sum(w[j].astype(F32).reshape(hs[c].shape) * hs[c], axis=0) for j in range(NT)]
                for st in stage[2 + N13 + c:3 + N13 + c]:
                    issue(st)
            if NV:
                out = jnp.concatenate([jnp.sum(v, axis=0, keepdims=True) for v in acc], axis=1)
            res = hres[0:1] + _r(out[0:1])
            o_v[...] = res.astype(o_v.dtype)
            pltpu.make_async_copy(o_v, o_hbm, sem_o).start()

        dma = pltpu.SemaphoreType.DMA
        pl.run_scoped(body, dma((R,)), dma((max(N13 + N2, 4),)))
        pltpu.make_async_copy(o_v, o_hbm, sem_o).wait()

    @jax.jit
    def run(A_x, A_k_cache, A_v_cache, A_wq, A_wo, B_x, B_w1, B_w3, B_w2):
        del B_x
        x = A_x.reshape(1, D)
        kt = jnp.swapaxes(A_k_cache.reshape(H, SK, DH), 1, 2)
        vt = jnp.swapaxes(A_v_cache.reshape(H, SK, DH), 1, 2)
        out = pl.pallas_call(
            kernel,
            out_shape=jax.ShapeDtypeStruct((1, D), A_x.dtype),
            in_specs=[pl.BlockSpec(memory_space=pl.ANY)] * 8,
            out_specs=pl.BlockSpec(memory_space=pl.ANY),
            scratch_shapes=[
                pltpu.VMEM((R, 2, DH, W), BF),
                pltpu.VMEM((D, H * DH), BF),
                pltpu.VMEM((H * DH * D // 1024, 8, 128), BF),
                pltpu.VMEM((3, GF, TF, 8, 128), BF),
                pltpu.VMEM((H, 8, DH), F32),
                pltpu.VMEM((1, D), BF),
                pltpu.VMEM((1, D), BF),
                pltpu.SemaphoreType.DMA(()),
            ],
            compiler_params=pltpu.CompilerParams(vmem_limit_bytes=64 * 1024 * 1024, disable_bounds_checks=True,
                                                 disable_semaphore_checks=True),
        )(x, kt, vt, A_wq, _tile_view(A_wo), *[_tile_view(w).reshape(GF, TF, 8, 128) for w in (B_w1, B_w3, B_w2)])
        return out.reshape(1, 1, D)

    return run


pallas_sequential_preLN__sliding_block_cached__glu_gated_swiglu__decode_kernel = make_kernel()
```

```python
import jax
import jax.numpy as jnp
import numpy as np
from jax import lax
import jax.experimental.pallas as pl
import jax.experimental.pallas.tpu as pltpu

H, DH, SK, D, F = 32, 192, 32768, 640, 1536
W = min(4096, max(256, SK // 4))
BF = jnp.bfloat16
F32 = jnp.float32


def _bf16_round(v):
    u = int(np.float32(v).view(np.uint32))
    u = (u + 0x7FFF + ((u >> 16) & 1)) & 0xFFFF0000
    return float(np.uint32(u).view(np.float32))


SCALE = _bf16_round(DH ** -0.5)
EPS = _bf16_round(1e-5)


def _r(x):
    return x.astype(BF).astype(F32)


def _layernorm(x32):
    m = jnp.mean(x32, axis=-1, keepdims=True)
    c = x32 - m
    v = jnp.mean(c * c, axis=-1, keepdims=True)
    num = _r(x32 - _r(m))
    den = _r(jnp.sqrt(_r(_r(v) + EPS)))
    return (num / den).astype(BF)


def _strided(n, groups):
    assert n % groups == 0
    return [g * (n // groups) + r for r in range(n // groups) for g in range(groups)]


def _zip2(a, b):
    assert len(a) == len(b)
    return [j for x, y in zip(a, b) for j in (x + (0,), y + (1,))]


def _alt(a):
    return [x + (i % 2,) for i, x in enumerate(a)]


def _split(lst, n):
    return [lst[i * len(lst) // n:(i + 1) * len(lst) // n] for i in range(n)]


def _schedule(jobs, ends, depth, ramp, lead):
    n = len(jobs)
    keyed = []
    for p, job in enumerate(jobs):
        if p >= n - depth:
            keyed.append((n - 3 * depth + 2 * (p - (n - depth)), job + (1,)))
        elif (n - depth - p) % 2:
            keyed.append((p, job + (0,)))
        else:
            keyed.append((p - 2 * depth * min(1.0, p / ramp), job + (1,)))
    keyed.sort(key=lambda kj: kj[0])
    cuts = [0] + [sum(k < e + lead for k, _ in keyed) for e in ends[:-1]] + [n]
    return [[j for _, j in keyed[a:b]] for a, b in zip(cuts, cuts[1:])]


def _kv_order(groups, mode, threads, shift):
    rows = _strided(DH // 8, groups)

    def order(rp):
        if mode == "h":
            return [(r, c) for c in (0, 1) for r in rp]
        if mode == "i":
            return [(r, c) for r in rp for c in (0, 1)]
        return [(r, (i + k) % 2) for k in (0, 1) for i, r in enumerate(rp)]

    k = [(0,) + p for p in order(rows)]
    v = [(1,) + p for p in order(rows[shift:] + rows[:shift])]
    if threads == "kv":
        return _zip2(k, v)
    if threads == "seq":
        return _alt(k + v)
    n = len(k) // 2
    return _zip2(k[:n], k[n:]) + _zip2(v[:n], v[n:])


def _tile_view(a):
    r, c = a.shape
    return a.reshape(r // 8, 8, c // 128, 128).transpose(0, 2, 1, 3).reshape(r * c // 1024, 8, 128)


def _untile(t, cols):
    nc = cols // 128
    t = t.reshape(t.shape[0] // nc, nc, 8, 128)
    return [t[:, j].reshape(t.shape[0] * 8, 128) for j in range(nc)]


def make_kernel(R=3, kv=(12, "h", "half", 22), qo=(5, 16), nq=2, n0=100, parts=4,
                f13=(4, 1, 16), N13=1, w2ch=((60, 1, 15),) * 3 + ((30, 1, 15), (15, 1, 15), (10, 2, 10), (5, 4, 5)),
                sched=(32, 96, 30), NV=3):
    QG, QT = qo
    GF, g13, t13 = f13
    TF = D * F // 1024 // GF
    T13 = TF // N13
    NT = D // 128
    N2 = len(w2ch)
    w2off = [sum(c[0] for c in w2ch[:i]) for i in range(N2)]
    assert (H * DH // 128) % QT == 0 and T13 % t13 == 0 and T13 % (F // 128) == 0
    assert sum(c[0] for c in w2ch) == TF and all(c[0] % NT == 0 for c in w2ch)
    kvp = _kv_order(*kv)
    HW = W // 2

    def kernel(x_hbm, kt_hbm, vt_hbm, wq_hbm, wo_hbm, w1_hbm, w3_hbm, w2_hbm, o_hbm,
               kv_v, wq_v, wo_v, wf_v, q_v, x_v, o_v, sem_kv, sems, sem_o):
        sem_x, sem_f, sem_wq, sem_wo = (sems.at[i] for i in range(4))

        def issue(jobs):
            for (src, dst, sem, idx, thread) in jobs:
                pltpu.make_async_copy(src.at[idx], dst.at[idx], sem).start(priority=thread)

        def wait_all(ref, sem):
            pltpu.make_async_copy(ref, ref, sem).wait()

        def head_jobs(h, slot):
            src = (kt_hbm.at[h, :, pl.ds(SK - W, W)], vt_hbm.at[h, :, pl.ds(SK - W, W)])
            return [(src[a], kv_v.at[slot, a], sem_kv.at[slot], (pl.ds(8 * r, 8), pl.ds(HW * c, HW)), t)
                    for a, r, c, t in kvp]

        x_copy = pltpu.make_async_copy(x_hbm, x_v, sem_x)
        x_copy.start()
        order = _strided(D * H * DH // 1024 // QT, QG)
        ppr = H * DH // 128 // QT
        jq = [(wq_hbm, wq_v, sem_f if p < ppr else sem_wq,
               (pl.ds(p // ppr * 8, 8), pl.ds(p % ppr * QT * 128, QT * 128))) for p in order]
        jo = [(wo_hbm, wo_v, sem_wo, (pl.ds(p * QT, QT),)) for p in order]
        issue(_zip2(jo, jq))
        wait_all(wq_v.at[pl.ds(0, 8)], sem_f)
        jobs = []
        for h in range(R - 1):
            jobs += head_jobs(h, h)
        issue(jobs[:n0])

        x_copy.wait()
        x32 = x_v[...].astype(F32)
        lnx = jnp.broadcast_to(_layernorm(x32), (8, D))
        wait_all(wq_v.at[pl.ds(8, D - 8)], sem_wq)
        QC = H // nq
        for c, group in enumerate(_split(jobs[n0:], nq)):
            qc = jnp.dot(lnx, wq_v[:, c * QC * DH:(c + 1) * QC * DH], preferred_element_type=F32)
            for j in range(QC):
                q_v[c * QC + j] = qc[:, j * DH:(j + 1) * DH]
            issue(group)
        wait_all(wo_v, sem_wo)

        def head_compute(h, slot, attn, jobs):
            groups = _split(jobs, 2 * parts)
            CW = W // parts
            wait_all(kv_v.at[slot], sem_kv.at[slot])
            qh = q_v[h].astype(BF)
            s = []
            for c in range(parts):
                s.append(jnp.dot(qh, kv_v[slot, 0, :, c * CW:(c + 1) * CW], preferred_element_type=F32))
                issue(groups[c])
            s = _r(_r(jnp.concatenate(s, axis=1)) * SCALE)
            m = jnp.max(s, axis=-1, keepdims=True)
            e = _r(jnp.exp(_r(s - m)))
            l = _r(jnp.sum(e, axis=-1, keepdims=True))
            p = (e / l).astype(BF)
            o = None
            for c in range(parts):
                o_ = lax.dot_general(p[:, c * CW:(c + 1) * CW], kv_v[slot, 1, :, c * CW:(c + 1) * CW],
                                     (((1,), (1,)), ((), ())), preferred_element_type=F32)
                o = o_ if o is None else o + o_
                issue(groups[parts + c])
            tph = DH // 8 * NT
            wo_h = jnp.concatenate(_untile(wo_v[pl.ds(h * tph, tph)], D), axis=1)
            return attn + jnp.dot(o.astype(BF), wo_h, preferred_element_type=F32)

        def head(h, attn):
            return head_compute(h, h % R, attn, head_jobs(h + R - 1, (h + R - 1) % R))

        attn = lax.fori_loop(0, H - R + 1, head, jnp.zeros((8, D), F32))

        tail, ends = [], []
        for c in range(N13):
            p13 = [(pl.ds(a, min(g13, GF - a)), pl.ds(c * T13 + t, t13))
                   for t in range(0, T13, t13) for a in range(0, GF, g13)]
            tail += [j for p in p13 for j in ((w1_hbm, wf_v.at[0], sems.at[c], p), (w3_hbm, wf_v.at[1], sems.at[c], p))]
            ends.append(len(tail))
        for c, (nt, g, t) in enumerate(w2ch):
            tail += [(w2_hbm, wf_v.at[2], sems.at[N13 + c],
                      (pl.ds(a, min(g, GF - a)), pl.ds(w2off[c] + u, min(t, nt - u))))
                     for u in range(0, nt, t) for a in range(0, GF, g)]
            ends.append(len(tail))
        stage = _schedule(tail, [0] + ends, *sched)
        for h in range(H - R + 1, H):
            attn = head_compute(h, h % R, attn, stage[h - H + 2] if h >= H - 2 else [])
        hres = _r(x32 + _r(attn))
        lnh = _layernorm(hres).astype(F32)

        def lhs(v, r0, nr):
            rg = v.shape[1] // GF
            return jnp.concatenate([v[:, a * rg + r0:a * rg + r0 + nr] for a in range(GF)], axis=1).astype(BF)

        def rhs(i, t0, nt, cols):
            return jnp.concatenate(_untile(wf_v[i, :, pl.ds(t0, nt)].reshape(GF * nt, 8, 128), cols), axis=1)

        R13 = D // GF // N13
        ls = [lhs(lnh, c * R13, R13) for c in range(N13)]
        gate = up = None
        for c in range(N13):
            wait_all(wf_v.at[pl.ds(0, 2), :, pl.ds(c * T13, T13)], sems.at[c])
            g_ = jnp.dot(ls[c], rhs(0, c * T13, T13, F), preferred_element_type=F32)
            u_ = jnp.dot(ls[c], rhs(1, c * T13, T13, F), preferred_element_type=F32)
            gate = g_ if gate is None else gate + g_
            up = u_ if up is None else up + u_
            issue(stage[2 + c])
        gate, up = _r(gate), _r(up)
        hm = _r(_r(gate * _r(jax.nn.sigmoid(gate))) * up)
        hs = [lhs(hm, w2off[c] // NT * 8, nt // NT * 8) for c, (nt, _, _) in enumerate(w2ch)]
        for c in range(N2 - NV, N2):
            nr = hs[c].shape[1]
            col = jnp.concatenate([hs[c][0:1].astype(F32), jnp.zeros((1, 128 - nr), F32)], axis=1)
            hs[c] = jnp.broadcast_to(col, (128, 128)).T[:nr].reshape(nr // 8, 8, 128)
        out = None
        for c, (nt, _, _) in enumerate(w2ch):
            if c == N2 - NV:
                first = lax.broadcasted_iota(jnp.int32, (8, 128), 0) == 0
                acc = [jnp.where(first, out[:, j * 128:(j + 1) * 128], 0.0) for j in range(NT)]
            wait_all(wf_v.at[2, :, pl.ds(w2off[c], nt)], sems.at[N13 + c])
            if c < N2 - NV:
                o_ = jnp.dot(hs[c], rhs(2, w2off[c], nt, D), preferred_element_type=F32)
                out = o_ if out is None else out + o_
            else:
                w = _untile(wf_v[2, :, pl.ds(w2off[c], nt)].reshape(GF * nt, 8, 128), D)
                acc = [acc[j] + jnp.sum(w[j].astype(F32).reshape(hs[c].shape) * hs[c], axis=0) for j in range(NT)]
            for st in stage[2 + N13 + c:3 + N13 + c]:
                issue(st)
        if NV:
            out = jnp.concatenate([jnp.sum(v, axis=0, keepdims=True) for v in acc], axis=1)
        res = hres[0:1] + _r(out[0:1])
        o_v[...] = res.astype(o_v.dtype)
        o_copy = pltpu.make_async_copy(o_v, o_hbm, sem_o)
        o_copy.start()
        o_copy.wait()

    @jax.jit
    def run(A_x, A_k_cache, A_v_cache, A_wq, A_wo, B_x, B_w1, B_w3, B_w2):
        del B_x
        x = A_x.reshape(1, D)
        kt = jnp.swapaxes(A_k_cache.reshape(H, SK, DH), 1, 2)
        vt = jnp.swapaxes(A_v_cache.reshape(H, SK, DH), 1, 2)
        out = pl.pallas_call(
            kernel,
            out_shape=jax.ShapeDtypeStruct((1, D), A_x.dtype),
            in_specs=[pl.BlockSpec(memory_space=pl.ANY)] * 8,
            out_specs=pl.BlockSpec(memory_space=pl.ANY),
            scratch_shapes=[
                pltpu.VMEM((R, 2, DH, W), BF),
                pltpu.VMEM((D, H * DH), BF),
                pltpu.VMEM((H * DH * D // 1024, 8, 128), BF),
                pltpu.VMEM((3, GF, TF, 8, 128), BF),
                pltpu.VMEM((H, 8, DH), F32),
                pltpu.VMEM((1, D), BF),
                pltpu.VMEM((1, D), BF),
                pltpu.SemaphoreType.DMA((R,)),
                pltpu.SemaphoreType.DMA((max(N13 + N2, 4),)),
                pltpu.SemaphoreType.DMA(()),
            ],
            compiler_params=pltpu.CompilerParams(vmem_limit_bytes=64 * 1024 * 1024, disable_bounds_checks=True,
                                                 disable_semaphore_checks=True),
        )(x, kt, vt, A_wq, _tile_view(A_wo), *[_tile_view(w).reshape(GF, TF, 8, 128) for w in (B_w1, B_w3, B_w2)])
        return out.reshape(1, 1, D)

    return run


pallas_sequential_preLN__sliding_block_cached__glu_gated_swiglu__decode_kernel = make_kernel()
```

```python
import jax
import jax.numpy as jnp
import numpy as np
from jax import lax
import jax.experimental.pallas as pl
import jax.experimental.pallas.tpu as pltpu

H, DH, SK, D, F = 32, 192, 32768, 640, 1536
W = min(4096, max(256, SK // 4))
BF = jnp.bfloat16
F32 = jnp.float32


def _bf16_round(v):
    u = int(np.float32(v).view(np.uint32))
    u = (u + 0x7FFF + ((u >> 16) & 1)) & 0xFFFF0000
    return float(np.uint32(u).view(np.float32))


SCALE = _bf16_round(DH ** -0.5)
EPS = _bf16_round(1e-5)


def _r(x):
    return x.astype(BF).astype(F32)


def _layernorm(x32):
    m = jnp.mean(x32, axis=-1, keepdims=True)
    c = x32 - m
    v = jnp.mean(c * c, axis=-1, keepdims=True)
    num = _r(x32 - _r(m))
    den = _r(jnp.sqrt(_r(_r(v) + EPS)))
    return (num / den).astype(BF)


def _strided(n, groups):
    assert n % groups == 0
    return [g * (n // groups) + r for r in range(n // groups) for g in range(groups)]


def _zip2(a, b):
    assert len(a) == len(b)
    return [j for x, y in zip(a, b) for j in (x + (0,), y + (1,))]


def _alt(a):
    return [x + (i % 2,) for i, x in enumerate(a)]


def _split(lst, n):
    return [lst[i * len(lst) // n:(i + 1) * len(lst) // n] for i in range(n)]


def _schedule(jobs, ends, depth, ramp, lead):
    n = len(jobs)
    keyed = []
    for p, job in enumerate(jobs):
        if p >= n - depth:
            keyed.append((n - 3 * depth + 2 * (p - (n - depth)), job + (1,)))
        elif (n - depth - p) % 2:
            keyed.append((p, job + (0,)))
        else:
            keyed.append((p - 2 * depth * min(1.0, p / ramp), job + (1,)))
    keyed.sort(key=lambda kj: kj[0])
    cuts = [0] + [sum(k < e + lead for k, _ in keyed) for e in ends[:-1]] + [n]
    return [[j for _, j in keyed[a:b]] for a, b in zip(cuts, cuts[1:])]


def _kv_order(groups, mode, threads, shift):
    rows = _strided(DH // 8, groups)

    def order(rp):
        if mode == "h":
            return [(r, c) for c in (0, 1) for r in rp]
        if mode == "i":
            return [(r, c) for r in rp for c in (0, 1)]
        return [(r, (i + k) % 2) for k in (0, 1) for i, r in enumerate(rp)]

    k = [(0,) + p for p in order(rows)]
    v = [(1,) + p for p in order(rows[shift:] + rows[:shift])]
    if threads == "kv":
        return _zip2(k, v)
    if threads == "seq":
        return _alt(k + v)
    n = len(k) // 2
    return _zip2(k[:n], k[n:]) + _zip2(v[:n], v[n:])


def _tile_view(a):
    r, c = a.shape
    return a.reshape(r // 8, 8, c // 128, 128).transpose(0, 2, 1, 3).reshape(r * c // 1024, 8, 128)


def _untile(t, cols):
    nc = cols // 128
    t = t.reshape(t.shape[0] // nc, nc, 8, 128)
    return [t[:, j].reshape(t.shape[0] * 8, 128) for j in range(nc)]


def make_kernel(R=3, kv=(12, "h", "half", 23), qo=(5, 16), nq=2, n0=100, parts=4,
                f13=(4, 1, 16), N13=1, w2ch=((80, 1, 16), (80, 1, 16), (50, 1, 17), (15, 1, 15), (10, 2, 10), (5, 4, 5)),
                sched=(32, 96, 30), NV=3):
    QG, QT = qo
    GF, g13, t13 = f13
    TF = D * F // 1024 // GF
    T13 = TF // N13
    NT = D // 128
    N2 = len(w2ch)
    w2off = [sum(c[0] for c in w2ch[:i]) for i in range(N2)]
    assert (H * DH // 128) % QT == 0 and T13 % t13 == 0 and T13 % (F // 128) == 0
    assert sum(c[0] for c in w2ch) == TF and all(c[0] % NT == 0 for c in w2ch)
    kvp = _kv_order(*kv)
    HW = W // 2

    def kernel(x_hbm, kt_hbm, vt_hbm, wq_hbm, wo_hbm, w1_hbm, w3_hbm, w2_hbm, o_hbm,
               kv_v, wq_v, wo_v, wf_v, q_v, x_v, o_v, sem_o):

        def body(sem_kv, sems):
            sem_x, sem_f, sem_wq, sem_wo = (sems.at[i] for i in range(4))

            def issue(jobs):
                for (src, dst, sem, idx, thread) in jobs:
                    pltpu.make_async_copy(src.at[idx], dst.at[idx], sem).start(priority=thread)

            def wait_all(ref, sem):
                pltpu.make_async_copy(ref, ref, sem).wait()

            def head_jobs(h, slot):
                src = (kt_hbm.at[h, :, pl.ds(SK - W, W)], vt_hbm.at[h, :, pl.ds(SK - W, W)])
                return [(src[a], kv_v.at[slot, a], sem_kv.at[slot], (pl.ds(8 * r, 8), pl.ds(HW * c, HW)), t)
                        for a, r, c, t in kvp]

            x_copy = pltpu.make_async_copy(x_hbm, x_v, sem_x)
            x_copy.start()
            order = _strided(D * H * DH // 1024 // QT, QG)
            ppr = H * DH // 128 // QT
            jq = [(wq_hbm, wq_v, sem_f if p < ppr else sem_wq,
                   (pl.ds(p // ppr * 8, 8), pl.ds(p % ppr * QT * 128, QT * 128))) for p in order]
            jo = [(wo_hbm, wo_v, sem_wo, (pl.ds(p * QT, QT),)) for p in order]
            issue(_zip2(jq, jo))
            wait_all(wq_v.at[pl.ds(0, 8)], sem_f)
            jobs = []
            for h in range(R - 1):
                jobs += head_jobs(h, h)
            issue(jobs[:n0])

            x_copy.wait()
            x32 = x_v[...].astype(F32)
            lnx = jnp.broadcast_to(_layernorm(x32), (8, D))
            wait_all(wq_v.at[pl.ds(8, D - 8)], sem_wq)
            QC = H // nq
            for c, group in enumerate(_split(jobs[n0:], nq)):
                qc = jnp.dot(lnx, wq_v[:, c * QC * DH:(c + 1) * QC * DH], preferred_element_type=F32)
                for j in range(QC):
                    q_v[c * QC + j] = qc[:, j * DH:(j + 1) * DH]
                issue(group)
            wait_all(wo_v, sem_wo)

            def head_compute(h, slot, attn, jobs):
                groups = _split(jobs, 2 * parts)
                CW = W // parts
                wait_all(kv_v.at[slot], sem_kv.at[slot])
                qh = q_v[h].astype(BF)
                s = []
                for c in range(parts):
                    s.append(jnp.dot(qh, kv_v[slot, 0, :, c * CW:(c + 1) * CW], preferred_element_type=F32))
                    issue(groups[c])
                s = _r(_r(jnp.concatenate(s, axis=1)) * SCALE)
                m = jnp.max(s, axis=-1, keepdims=True)
                e = _r(jnp.exp(_r(s - m)))
                l = _r(jnp.sum(e, axis=-1, keepdims=True))
                p = (e / l).astype(BF)
                o = None
                for c in range(parts):
                    o_ = lax.dot_general(p[:, c * CW:(c + 1) * CW], kv_v[slot, 1, :, c * CW:(c + 1) * CW],
                                         (((1,), (1,)), ((), ())), preferred_element_type=F32)
                    o = o_ if o is None else o + o_
                    issue(groups[parts + c])
                tph = DH // 8 * NT
                wo_h = jnp.concatenate(_untile(wo_v[pl.ds(h * tph, tph)], D), axis=1)
                return attn + jnp.dot(o.astype(BF), wo_h, preferred_element_type=F32)

            def head(h, attn):
                return head_compute(h, h % R, attn, head_jobs(h + R - 1, (h + R - 1) % R))

            attn = lax.fori_loop(0, H - R + 1, head, jnp.zeros((8, D), F32))

            tail, ends = [], []
            for c in range(N13):
                p13 = [(pl.ds(a, min(g13, GF - a)), pl.ds(c * T13 + t, t13))
                       for t in range(0, T13, t13) for a in range(0, GF, g13)]
                tail += [j for p in p13 for j in ((w1_hbm, wf_v.at[0], sems.at[c], p), (w3_hbm, wf_v.at[1], sems.at[c], p))]
                ends.append(len(tail))
            for c, (nt, g, t) in enumerate(w2ch):
                tail += [(w2_hbm, wf_v.at[2], sems.at[N13 + c],
                          (pl.ds(a, min(g, GF - a)), pl.ds(w2off[c] + u, min(t, nt - u))))
                         for u in range(0, nt, t) for a in range(0, GF, g)]
                ends.append(len(tail))
            stage = _schedule(tail, [0] + ends, *sched)
            for h in range(H - R + 1, H):
                attn = head_compute(h, h % R, attn, stage[h - H + 2] if h >= H - 2 else [])
            hres = _r(x32 + _r(attn))
            lnh = _layernorm(hres).astype(F32)

            def lhs(v, r0, nr):
                rg = v.shape[1] // GF
                return jnp.concatenate([v[:, a * rg + r0:a * rg + r0 + nr] for a in range(GF)], axis=1).astype(BF)

            def rhs(i, t0, nt, cols):
                return jnp.concatenate(_untile(wf_v[i, :, pl.ds(t0, nt)].reshape(GF * nt, 8, 128), cols), axis=1)

            R13 = D // GF // N13
            ls = [lhs(lnh, c * R13, R13) for c in range(N13)]
            gate = up = None
            for c in range(N13):
                wait_all(wf_v.at[pl.ds(0, 2), :, pl.ds(c * T13, T13)], sems.at[c])
                g_ = jnp.dot(ls[c], rhs(0, c * T13, T13, F), preferred_element_type=F32)
                u_ = jnp.dot(ls[c], rhs(1, c * T13, T13, F), preferred_element_type=F32)
                gate = g_ if gate is None else gate + g_
                up = u_ if up is None else up + u_
                issue(stage[2 + c])
            gate, up = _r(gate), _r(up)
            hm = _r(_r(gate * _r(jax.nn.sigmoid(gate))) * up)
            hs = [lhs(hm, w2off[c] // NT * 8, nt // NT * 8) for c, (nt, _, _) in enumerate(w2ch)]
            for c in range(N2 - NV, N2):
                nr = hs[c].shape[1]
                col = jnp.concatenate([hs[c][0:1].astype(F32), jnp.zeros((1, 128 - nr), F32)], axis=1)
                hs[c] = jnp.broadcast_to(col, (128, 128)).T[:nr].reshape(nr // 8, 8, 128)
            out = None
            for c, (nt, _, _) in enumerate(w2ch):
                if c == N2 - NV:
                    first = lax.broadcasted_iota(jnp.int32, (8, 128), 0) == 0
                    acc = [jnp.where(first, out[:, j * 128:(j + 1) * 128], 0.0) for j in range(NT)]
                wait_all(wf_v.at[2, :, pl.ds(w2off[c], nt)], sems.at[N13 + c])
                if c < N2 - NV:
                    o_ = jnp.dot(hs[c], rhs(2, w2off[c], nt, D), preferred_element_type=F32)
                    out = o_ if out is None else out + o_
                else:
                    w = _untile(wf_v[2, :, pl.ds(w2off[c], nt)].reshape(GF * nt, 8, 128), D)
                    acc = [acc[j] + jnp.sum(w[j].astype(F32).reshape(hs[c].shape) * hs[c], axis=0) for j in range(NT)]
                for st in stage[2 + N13 + c:3 + N13 + c]:
                    issue(st)
            if NV:
                out = jnp.concatenate([jnp.sum(v, axis=0, keepdims=True) for v in acc], axis=1)
            res = hres[0:1] + _r(out[0:1])
            o_v[...] = res.astype(o_v.dtype)
            pltpu.make_async_copy(o_v, o_hbm, sem_o).start()

        dma = pltpu.SemaphoreType.DMA
        pl.run_scoped(body, dma((R,)), dma((max(N13 + N2, 4),)))
        pltpu.make_async_copy(o_v, o_hbm, sem_o).wait()

    @jax.jit
    def run(A_x, A_k_cache, A_v_cache, A_wq, A_wo, B_x, B_w1, B_w3, B_w2):
        del B_x
        x = A_x.reshape(1, D)
        kt = jnp.swapaxes(A_k_cache.reshape(H, SK, DH), 1, 2)
        vt = jnp.swapaxes(A_v_cache.reshape(H, SK, DH), 1, 2)
        out = pl.pallas_call(
            kernel,
            out_shape=jax.ShapeDtypeStruct((1, D), A_x.dtype),
            in_specs=[pl.BlockSpec(memory_space=pl.ANY)] * 8,
            out_specs=pl.BlockSpec(memory_space=pl.ANY),
            scratch_shapes=[
                pltpu.VMEM((R, 2, DH, W), BF),
                pltpu.VMEM((D, H * DH), BF),
                pltpu.VMEM((H * DH * D // 1024, 8, 128), BF),
                pltpu.VMEM((3, GF, TF, 8, 128), BF),
                pltpu.VMEM((H, 8, DH), F32),
                pltpu.VMEM((1, D), BF),
                pltpu.VMEM((1, D), BF),
                pltpu.SemaphoreType.DMA(()),
            ],
            compiler_params=pltpu.CompilerParams(vmem_limit_bytes=64 * 1024 * 1024, disable_bounds_checks=True,
                                                 disable_semaphore_checks=True),
        )(x, kt, vt, A_wq, _tile_view(A_wo), *[_tile_view(w).reshape(GF, TF, 8, 128) for w in (B_w1, B_w3, B_w2)])
        return out.reshape(1, 1, D)

    return run


pallas_sequential_preLN__sliding_block_cached__glu_gated_swiglu__decode_kernel = make_kernel()
```
